```python
import jax
import jax.numpy as jnp

def _softmax(x, axis=-1):
    return jax.nn.softmax(x, axis=axis)
def _gelu(x):
    return jax.nn.gelu(x, approximate=True)
def _silu(x):
    return jax.nn.silu(x)
def _sigmoid(x):
    return jax.nn.sigmoid(x)
def _layernorm(x, axis=-1, eps=1e-5):
    m = jnp.mean(x, axis=axis, keepdims=True)
    v = jnp.var(x, axis=axis, keepdims=True)
    return (x - m) / jnp.sqrt(v + eps)
def _scatter_add(tgt, idx, src, axis=0):
    return tgt.at[idx].add(src)
def _segment_sum(src, seg, n):
    return jax.ops.segment_sum(src, seg, n)
class _Rng:
    def __init__(self, key):
        self._k = key
    def _next(self):
        self._k, sub = jax.random.split(self._k)
        return sub
    def normal(self, shape):
        return jax.random.normal(self._next(), shape, dtype=jnp.bfloat16)
    def randint(self, lo, hi, shape):
        return jax.random.randint(self._next(), shape, lo, hi, dtype=jnp.int32)
    def uniform(self, shape, lo=0.0, hi=1.0):
        return jax.random.uniform(self._next(), shape, jnp.bfloat16, lo, hi)
    def permutation(self, n):
        return jax.random.permutation(self._next(), n)


kernel_name = 'sequential_preLN__sliding_block_cached__mixer_s_mlp__decode'

def setup_inputs():
    _rng = _Rng(jax.random.key(int.from_bytes(__import__("os").urandom(4), "little")))
    _w = (lambda a: (lambda t: t.astype(jnp.bfloat16) if jnp.issubdtype(t.dtype, jnp.floating) else t)(jnp.asarray(a)))
    def _A_setup():
        B, Sq, D = 1, 1, 640
        Hq, Hkv, Sk, Dh = 32, 32, 32768, 192
        assert Hq % Hkv == 0, (Hq, Hkv)
        return {
            "x": _w((lambda *s: _rng.normal(s) * 0.05)(B, Sq, D)),
            "k_cache": _w((lambda *s: _rng.normal(s) * 0.05)(B, Hkv, Sk, Dh)),
            "v_cache": _w((lambda *s: _rng.normal(s) * 0.05)(B, Hkv, Sk, Dh)),
            "wq": _w((lambda *s: _rng.normal(s) * 0.05)(D, Hq * Dh) * (D ** -0.5)),
            "wo": _w((lambda *s: _rng.normal(s) * 0.05)(Hq * Dh, D) * ((Hq * Dh) ** -0.5)),
        }
    _A_in = _A_setup()

    def _B_setup():
        B, S, D, F = 1, 1, 640, 1536
        return {
            "x":  _w((lambda *s: _rng.normal(s) * 0.05)(B, S, D)),
            "w1": _w((lambda *s: _rng.normal(s) * 0.05)(D, D) * (D ** -0.5)),
            "w2": _w((lambda *s: _rng.normal(s) * 0.05)(D, D) * (D ** -0.5)),
            "w3": _w((lambda *s: _rng.normal(s) * 0.05)(D, F) * (D ** -0.5)),
            "w4": _w((lambda *s: _rng.normal(s) * 0.05)(F, D) * (F ** -0.5)),
        }
    _B_in = _B_setup()

    return {
        "A_x": _A_in["x"],
        "A_k_cache": _A_in["k_cache"],
        "A_v_cache": _A_in["v_cache"],
        "A_wq": _A_in["wq"],
        "A_wo": _A_in["wo"],
        "B_x": _B_in["x"],
        "B_w1": _B_in["w1"],
        "B_w2": _B_in["w2"],
        "B_w3": _B_in["w3"],
        "B_w4": _B_in["w4"],
    }

def reference(A_x, A_k_cache, A_v_cache, A_wq, A_wo, B_x, B_w1, B_w2, B_w3, B_w4):
    def _A_ref(x, k_cache, v_cache, wq, wo):
        B, Sq, D = x.shape
        Hq, Dh = 32, 192
        Hkv, Sk = k_cache.shape[1], k_cache.shape[2]
        W = min(4096, max(256, Sk // 4))
        rep = Hq // Hkv
        q = (lambda x, *d: x.transpose(*d))((x @ wq).reshape(B, Sq, Hq, Dh), 0, 2, 1, 3)
        k = jnp.repeat(k_cache[:, :, Sk - W:, :], rep, axis=1)
        v = jnp.repeat(v_cache[:, :, Sk - W:, :], rep, axis=1)
        scores = jnp.einsum("bhqd,bhkd->bhqk", q, k) * (Dh ** -0.5)
        p = _softmax(scores, axis=-1)
        o = jnp.einsum("bhqk,bhkd->bhqd", p, v)
        return (lambda x, *d: x.transpose(*d))(o, 0, 2, 1, 3).reshape(B, Sq, Hq * Dh) @ wo

    def _B_ref(x, w1, w2, w3, w4):
        B, S, D = x.shape
        h = _gelu(_layernorm(x, axis=-1) @ w1)
        c = D // 4
        g0 = jnp.pad(h[:, :, 0*c:1*c], ((0, 0), (1, 0), (0, 0)))[:, :S, :]
        g1 = jnp.pad(h[:, :, 1*c:2*c], ((0, 0), (0, 1), (0, 0)))[:, 1:, :]
        g2 = jnp.pad(h[:, :, 2*c:3*c], ((0, 0), (2, 0), (0, 0)))[:, :S, :]
        g3 = jnp.pad(h[:, :, 3*c:   ], ((0, 0), (0, 2), (0, 0)))[:, 2:, :]
        hs = jnp.concatenate([g0, g1, g2, g3], axis=-1) @ w2
        x1 = x + hs
        h2 = _gelu(_layernorm(x1, axis=-1) @ w3) @ w4
        return x1 + h2

    x = A_x
    h = x + _A_ref(_layernorm(x, axis=-1), A_k_cache, A_v_cache, A_wq, A_wo)
    h2 = h + _B_ref(_layernorm(h, axis=-1), B_w1, B_w2, B_w3, B_w4)
    return h2
```

```python
import jax
import jax.numpy as jnp
from jax import lax
import jax.experimental.pallas as pl
import jax.experimental.pallas.tpu as pltpu

F32 = jnp.float32
BF16 = jnp.bfloat16

EPS = 1e-5
CL = 256
NSLOT = 32
DEPTH = 16
P_BULK = 1
P_SMALL = 0
WQ_ROWS = 16
WO_ROWS = 16
QK_MODE = "vpu"


def _ln(v):
    m = jnp.mean(v, axis=-1, keepdims=True)
    c = v - m
    var = jnp.mean(c * c, axis=-1, keepdims=True)
    return c / jnp.sqrt(var + EPS)


def _make_kernel(H, DH, SK, W, D, FF):
    NCH = W // CL
    assert NSLOT == 2 * NCH
    W0 = SK - W
    PW = 2 * DH
    NPAIR = H // 2
    NWQ = D // WQ_ROWS
    NWO = DH // WO_ROWS
    scale = float(DH) ** -0.5

    W3_ROWS = 16
    NW3 = D // W3_ROWS
    W4_ROWS = FF // DEPTH
    assert W4_ROWS * DEPTH == FF and W4_ROWS % 16 == 0
    W4_GROUPS = 4
    W4_PER_GROUP = DEPTH // W4_GROUPS

    def kernel(x_hbm, kt_hbm, vt_hbm, wq_hbm, wo_hbm, w3_hbm, w4_hbm, out_ref,
               ring, wq_buf, wo_buf, w3_buf, w4_buf, x_buf, xn_ref, qb_ref,
               s_ref, acc_ref, y_ref,
               ring_sem, wq_sem, wo_sem, w3_sem, w4_sem, x_sem):

        def chunk_copy(h, t):
            src = kt_hbm if t < NCH else vt_hbm
            c = t % NCH
            return pltpu.make_async_copy(
                src.at[h, :, pl.ds(W0 + c * CL, CL)], ring.at[t], ring_sem.at[t])

        def chunk_wait(t):
            pltpu.make_async_copy(ring.at[t], ring.at[t], ring_sem.at[t]).wait()

        def wq_copy(pair, i):
            col = pair * PW
            if not isinstance(col, int):
                col = pl.multiple_of(col, 128)
            return pltpu.make_async_copy(
                wq_hbm.at[pl.ds(i * WQ_ROWS, WQ_ROWS), pl.ds(col, PW)],
                wq_buf.at[pl.ds(i * WQ_ROWS, WQ_ROWS), :], wq_sem.at[0])

        def wo_copy(h, par, i):
            row = h * DH + i * WO_ROWS
            if not isinstance(row, int):
                row = pl.multiple_of(row, 16)
            return pltpu.make_async_copy(
                wo_hbm.at[pl.ds(row, WO_ROWS), :],
                wo_buf.at[par, pl.ds(i * WO_ROWS, WO_ROWS), :], wo_sem.at[par])

        def w3_copy(i):
            return pltpu.make_async_copy(
                w3_hbm.at[pl.ds(i * W3_ROWS, W3_ROWS), :],
                w3_buf.at[pl.ds(i * W3_ROWS, W3_ROWS), :], w3_sem.at[0])

        def w4_copy(i):
            return pltpu.make_async_copy(
                w4_hbm.at[pl.ds(i * W4_ROWS, W4_ROWS), :],
                w4_buf.at[pl.ds(i * W4_ROWS, W4_ROWS), :],
                w4_sem.at[i // W4_PER_GROUP])

        def wait_all(buf, sem):
            pltpu.make_async_copy(buf, buf, sem).wait()

        def q_tile(j):
            q = jnp.dot(xn_ref[...], wq_buf[:, j * 128:(j + 1) * 128],
                        preferred_element_type=F32)
            q = q.astype(BF16).astype(F32) * scale
            qb_ref[j * 128:(j + 1) * 128, :] = jnp.broadcast_to(q[0:1, :], (128, 128)).T

        def oproj_piece(par, i, inv_l, y):
            r0 = i * WO_ROWS
            o = jnp.sum(acc_ref[r0:r0 + WO_ROWS, :], axis=1, keepdims=True) * inv_l
            pr = wo_buf[par, r0:r0 + WO_ROWS, :].astype(F32) * o
            for g in range(WO_ROWS // 8):
                y = y + pr[g * 8:(g + 1) * 8, :]
            return y

        def load_inv_l():
            l = jnp.sum(acc_ref[DH:DH + 1, :], axis=1, keepdims=True)
            return 1.0 / l

        def head(h, par, issue_bulk, issue_small, side):
            qb = qb_ref[par * DH:(par + 1) * DH, :]
            qb2 = jnp.concatenate([qb] * (CL // 128), axis=1)
            m_vec = None
            inv_l = None
            y = None
            for t in range(NCH):
                chunk_wait(t)
                issue_bulk(t)
                issue_small(t)
                kt = ring[t].astype(F32)
                s = jnp.sum(kt * qb2, axis=0, keepdims=True)
                s_ref[:, t * CL:(t + 1) * CL] = s
                m_vec = s if m_vec is None else jnp.maximum(m_vec, s)
                if t == 0:
                    inv_l = load_inv_l()
                    y = y_ref[...]
                if t < NWO:
                    y = oproj_piece(1 - par, t, inv_l, y)
                if t == NWO - 1:
                    y_ref[...] = y
                for fn in side.get(t, ()):
                    fn()
            acc = None
            l_vec = None
            m = None
            for c in range(NCH):
                t = NCH + c
                chunk_wait(t)
                issue_bulk(t)
                issue_small(t)
                if c == 0:
                    m = jnp.max(m_vec, axis=1, keepdims=True)
                p = jnp.exp(s_ref[:, c * CL:(c + 1) * CL] - m)
                pr = ring[t].astype(F32) * p
                for g in range(CL // 128):
                    pg = pr[:, g * 128:(g + 1) * 128]
                    acc = pg if acc is None else acc + pg
                    lg = p[:, g * 128:(g + 1) * 128]
                    l_vec = lg if l_vec is None else l_vec + lg
                for fn in side.get(t, ()):
                    fn()
            acc_ref[0:DH, :] = acc
            acc_ref[DH:DH + 8, :] = jnp.broadcast_to(l_vec, (8, 128))

        def pair_body(pair, last):
            ha = 2 * pair
            hb = ha + 1

            def bulk(h, is_last_head):
                def issue(t):
                    tt = t + DEPTH
                    if tt < NSLOT:
                        chunk_copy(h, tt).start(priority=P_BULK)
                    elif not is_last_head:
                        chunk_copy(h + 1, tt - NSLOT).start(priority=P_BULK)
                    else:
                        w4_copy(tt - NSLOT).start(priority=P_BULK)
                return issue

            sched = [None] * (2 * NSLOT)
            wq_slots = list(range(0, 16)) + list(range(28, 52))
            for i, u in enumerate(wq_slots):
                if last:
                    sched[u] = (lambda i=i: w3_copy(i))
                else:
                    sched[u] = (lambda i=i: wq_copy(pair + 1, i))
            for i in range(NWO):
                sched[16 + i] = (lambda i=i: wo_copy(hb, 1, i))
                if not last:
                    sched[52 + i] = (lambda i=i: wo_copy(ha + 2, 0, i))

            def small(base):
                def issue(t):
                    fn = sched[base + t]
                    if fn is not None:
                        fn().start(priority=P_SMALL)
                return issue

            side_a = {NSLOT - 1: [lambda: wait_all(wo_buf.at[0], wo_sem.at[0])]}
            side_b = {NSLOT - 1: [lambda: wait_all(wo_buf.at[1], wo_sem.at[1])]}
            if not last:
                side_b[24] = [lambda: wait_all(wq_buf, wq_sem.at[0]), lambda: q_tile(0)]
                side_b[26] = [lambda: q_tile(1)]
                side_b[28] = [lambda: q_tile(2)]
            head(ha, 0, bulk(ha, False), small(0), side_a)
            head(hb, 1, bulk(hb, last), small(NSLOT), side_b)

        x_cp = pltpu.make_async_copy(x_hbm, x_buf, x_sem.at[0])
        x_cp.start(priority=P_SMALL)
        wq0 = pltpu.make_async_copy(wq_hbm.at[:, pl.ds(0, PW)], wq_buf, wq_sem.at[0])
        wq0.start(priority=P_SMALL)
        for t in range(DEPTH):
            chunk_copy(0, t).start(priority=P_BULK)
        pltpu.make_async_copy(wo_hbm.at[pl.ds(0, DH), :], wo_buf.at[0],
                              wo_sem.at[0]).start(priority=P_BULK)

        acc_ref[0:DH, :] = jnp.zeros((DH, 128), F32)
        acc_ref[DH:DH + 8, :] = jnp.ones((8, 128), F32)
        wo_buf[1] = jnp.zeros((DH, D), BF16)
        y_ref[...] = jnp.zeros((8, D), F32)

        x_cp.wait()
        x = x_buf[...].astype(F32)
        xn_ref[...] = jnp.broadcast_to(_ln(x), (8, D)).astype(BF16)
        wq0.wait()
        for j in range(PW // 128):
            q_tile(j)

        def loop_body(pair, carry):
            pair_body(pair, False)
            return carry

        lax.fori_loop(0, NPAIR - 1, loop_body, 0)
        pair_body(NPAIR - 1, True)

        inv_l = load_inv_l()
        y = y_ref[...]
        for i in range(NWO):
            y = oproj_piece(1, i, inv_l, y)
        attn = jnp.sum(y, axis=0, keepdims=True)
        h = x_buf[...].astype(F32) + attn
        x1 = _ln(h)
        yn = jnp.broadcast_to(_ln(x1), (8, D)).astype(BF16)
        wait_all(w3_buf, w3_sem.at[0])
        g = jnp.dot(yn, w3_buf[...], preferred_element_type=F32)
        g = jax.nn.gelu(g, approximate=True).astype(BF16)
        res = h + x1
        gr = W4_PER_GROUP * W4_ROWS
        h2 = None
        for k in range(W4_GROUPS):
            wait_all(w4_buf.at[pl.ds(k * gr, gr), :], w4_sem.at[k])
            part = jnp.dot(g[:, k * gr:(k + 1) * gr], w4_buf[k * gr:(k + 1) * gr, :],
                           preferred_element_type=F32)
            h2 = part if h2 is None else h2 + part
        out_ref[...] = (res + h2[0:1, :]).astype(out_ref.dtype)

    scratch = [
        pltpu.VMEM((NSLOT, DH, CL), BF16),
        pltpu.VMEM((D, PW), BF16),
        pltpu.VMEM((2, DH, D), BF16),
        pltpu.VMEM((D, FF), BF16),
        pltpu.VMEM((FF, D), BF16),
        pltpu.VMEM((1, D), BF16),
        pltpu.VMEM((8, D), BF16),
        pltpu.VMEM((PW, 128), F32),
        pltpu.VMEM((1, W), F32),
        pltpu.VMEM((DH + 8, 128), F32),
        pltpu.VMEM((8, D), F32),
        pltpu.SemaphoreType.DMA((NSLOT,)),
        pltpu.SemaphoreType.DMA((1,)),
        pltpu.SemaphoreType.DMA((2,)),
        pltpu.SemaphoreType.DMA((1,)),
        pltpu.SemaphoreType.DMA((W4_GROUPS,)),
        pltpu.SemaphoreType.DMA((1,)),
    ]
    return kernel, scratch


@jax.jit
def pallas_sequential_preLN__sliding_block_cached__mixer_s_mlp__decode_kernel(
    A_x: jax.Array,
    A_k_cache: jax.Array,
    A_v_cache: jax.Array,
    A_wq: jax.Array,
    A_wo: jax.Array,
    B_x: jax.Array,
    B_w1: jax.Array,
    B_w2: jax.Array,
    B_w3: jax.Array,
    B_w4: jax.Array,
):
    B, S, D = A_x.shape
    _, H, SK, DH = A_k_cache.shape
    FF = B_w3.shape[1]
    assert B == 1 and S == 1
    W = min(4096, max(256, SK // 4))

    kt = jnp.swapaxes(A_k_cache, 2, 3).reshape(H, DH, SK)
    vt = jnp.swapaxes(A_v_cache, 2, 3).reshape(H, DH, SK)
    x2 = A_x.reshape(1, D)

    kernel, scratch = _make_kernel(H, DH, SK, W, D, FF)
    out = pl.pallas_call(
        kernel,
        in_specs=[pl.BlockSpec(memory_space=pl.ANY)] * 7,
        out_specs=pl.BlockSpec(memory_space=pltpu.VMEM),
        out_shape=jax.ShapeDtypeStruct((1, D), A_x.dtype),
        scratch_shapes=scratch,
        compiler_params=pltpu.CompilerParams(
            vmem_limit_bytes=32 * 1024 * 1024,
            disable_bounds_checks=True,
        ),
    )(x2, kt, vt, A_wq, A_wo, B_w3, B_w4)
    return out.reshape(B, S, D)
```

```python
import jax
import jax.numpy as jnp
from jax import lax
import jax.experimental.pallas as pl
import jax.experimental.pallas.tpu as pltpu

F32 = jnp.float32
BF16 = jnp.bfloat16

EPS = 1e-5
CL = 256
P_BULK = 1
P_SMALL = 0
OR = 16
W4_EARLY = (192, 192)
W4_TAIL_ROWS = 128
W4_MXU_GROUPS = (1152, 256)
W4_VPU_GROUPS = (64, 64)


def _ln(v):
    m = jnp.mean(v, axis=-1, keepdims=True)
    c = v - m
    var = jnp.mean(c * c, axis=-1, keepdims=True)
    return c / jnp.sqrt(var + EPS)


def _pieces640(r_lo, r_hi):
    out = []
    for r in range(r_lo, r_hi, 64):
        out += [(r + i * 16, 16, 0, 512) for i in range(4)] + [(r, 64, 512, 128)]
    return out


def _col_bcast(row):
    eye = (lax.broadcasted_iota(jnp.int32, (128, 128), 0)
           == lax.broadcasted_iota(jnp.int32, (128, 128), 1))
    col = jnp.sum(jnp.where(eye, jnp.broadcast_to(row, (128, 128)), 0.0),
                  axis=1, keepdims=True)
    return jnp.broadcast_to(col, (128, 128))


def _make_kernel(H, DH, SK, W, D, FF):
    NCH = W // CL
    W0 = SK - W
    HD = H * DH
    NOP = DH // OR
    NQT = HD // 128
    scale = float(DH) ** -0.5
    assert (H, DH, NCH, D, FF) == (32, 192, 16, 640, 1536)

    wo_pcs = _pieces640(0, DH)
    e1_pcs = _pieces640(0, W4_EARLY[0])
    e2_pcs = _pieces640(W4_EARLY[0], sum(W4_EARLY))
    groups, r = [], 0
    for n in W4_MXU_GROUPS + W4_VPU_GROUPS:
        groups.append((r, n))
        r += n
    assert r == FF
    NM = len(W4_MXU_GROUPS)
    V0 = groups[NM][0]
    tail_pcs = []
    for k, (g0, n) in enumerate(groups):
        r = max(g0, sum(W4_EARLY))
        while r < g0 + n:
            nr = min(W4_TAIL_ROWS, g0 + n - r)
            tail_pcs.append((r, nr, k))
            r += nr
    assert len(tail_pcs) <= NCH

    def kernel(x_hbm, kt_hbm, vt_hbm, wq_hbm, wo_hbm, w3_hbm, w4_hbm, out_ref,
               kbuf, vbuf, wq_buf, wo_buf, w3_buf, w4_buf, x_buf, xn_ref, qb_ref,
               s_ref, acc_ref, y_ref,
               c_sem, wq_sem, wo_sem, w3_sem, w4_sem, x_sem):

        def al(v, m):
            return v if isinstance(v, int) else pl.multiple_of(v, m)

        def k_copy(h, c):
            return pltpu.make_async_copy(
                kt_hbm.at[h, :, pl.ds(al(W0 + c * CL, CL), CL)], kbuf.at[h, c],
                c_sem.at[c])

        def v_copy(h, c):
            return pltpu.make_async_copy(
                vt_hbm.at[h, :, pl.ds(W0 + c * CL, CL)], vbuf.at[h % 2, c],
                c_sem.at[c])

        def wait_all(buf, sem):
            pltpu.make_async_copy(buf, buf, sem).wait()

        def wq_copy(rg, lb, lanes):
            row = al(rg * 8, 8)
            return pltpu.make_async_copy(
                wq_hbm.at[pl.ds(row, 8), pl.ds(lb * lanes, lanes)],
                wq_buf.at[pl.ds(row, 8), pl.ds(lb * lanes, lanes)], wq_sem.at[0])

        def wo_copy(h, pc):
            r0, nr, c0, nc = pc
            row = al(h * DH + r0, 16)
            return pltpu.make_async_copy(
                wo_hbm.at[pl.ds(row, nr), pl.ds(c0, nc)],
                wo_buf.at[h + 1, pl.ds(r0, nr), pl.ds(c0, nc)], wo_sem.at[h % 2])

        def w3_copy(i):
            row = al(i * 8, 8)
            return pltpu.make_async_copy(
                w3_hbm.at[pl.ds(row, 8), :], w3_buf.at[pl.ds(row, 8), :],
                w3_sem.at[0])

        def w4_copy(pc, k):
            r0, nr, c0, nc = pc
            return pltpu.make_async_copy(
                w4_hbm.at[pl.ds(r0, nr), pl.ds(c0, nc)],
                w4_buf.at[pl.ds(r0, nr), pl.ds(c0, nc)], w4_sem.at[k])

        def k_step(h, c):
            wait_all(kbuf.at[h, c], c_sem.at[c])
            k_copy(h + 1, c).start(priority=P_BULK)

        def q_row(j):
            col = al(j * 128, 128)
            q = jnp.dot(xn_ref[...], wq_buf[:, pl.ds(col, 128)],
                        preferred_element_type=F32)
            return q.astype(BF16).astype(F32) * scale

        def oproj_piece(slot, i, inv_l, y):
            r0 = i * OR
            o = jnp.sum(acc_ref[r0:r0 + OR, :], axis=1, keepdims=True) * inv_l
            pr = wo_buf[slot, r0:r0 + OR, :].astype(F32) * o
            for g in range(OR // 8):
                y = y + pr[g * 8:(g + 1) * 8, :]
            return y

        def load_inv_l():
            l = jnp.sum(acc_ref[DH:DH + 1, :], axis=1, keepdims=True)
            return 1.0 / l

        def load_qb(h):
            qb = qb_ref[pl.ds(al(h * DH, 64), DH), :]
            return jnp.concatenate([qb] * (CL // 128), axis=1)

        def qk_step(h, c, qb2, m_vec):
            s = jnp.sum(kbuf[h, c].astype(F32) * qb2, axis=0, keepdims=True)
            s_ref[h % 2, :, c * CL:(c + 1) * CL] = s
            return s if m_vec is None else jnp.maximum(m_vec, s)

        x_cp = pltpu.make_async_copy(x_hbm, x_buf, x_sem.at[0])
        x_cp.start(priority=P_SMALL)
        for c in range(NCH):
            k_copy(0, c).start(priority=P_BULK)

        acc_ref[0:DH, :] = jnp.zeros((DH, 128), F32)
        acc_ref[DH:DH + 8, :] = jnp.ones((8, 128), F32)
        wo_buf[0] = jnp.zeros((DH, D), BF16)
        y_ref[...] = jnp.zeros((8, D), F32)

        def a_body(it, carry):
            for u in range(3 * NCH):
                k_step(it * 3 + u // NCH, u % NCH)
                wq_copy(it * 8 + u // 6, u % 6, 1024).start(priority=P_SMALL)
            return carry

        lax.fori_loop(0, 8, a_body, 0)
        for u in range(3 * NCH):
            k_step(24 + u // NCH, u % NCH)
            wq_copy(64 + u // 3, u % 3, 2048).start(priority=P_SMALL)

        e1 = list(e1_pcs)

        def e1_slot():
            if e1:
                w4_copy(e1.pop(0), 0).start(priority=P_SMALL)

        HQ = 27
        q0 = None
        for u in range(5):
            k_step(HQ, u)
            e1_slot()
            if u == 0:
                x_cp.wait()
                xn = _ln(x_buf[...].astype(F32))
                xn_ref[...] = jnp.broadcast_to(xn, (8, D)).astype(BF16)
            if u == 4:
                wait_all(wq_buf, wq_sem.at[0])
                q0 = q_row(0)

        def q_body(i, q):
            u = i + 5
            k_step(HQ + u // NCH, u % NCH)
            w3_copy(i).start(priority=P_SMALL)
            qb_ref[pl.ds(al(i * 128, 128), 128), :] = _col_bcast(q[0:1, :])
            return q_row(jnp.minimum(i + 1, NQT - 1))

        lax.fori_loop(0, NQT, q_body, q0)
        for u in range(5 + NQT, 4 * NCH):
            k_step(HQ + u // NCH, u % NCH)
            e1_slot()

        m_vec = None
        qb2 = load_qb(0)
        for c in range(NCH):
            wait_all(kbuf.at[H - 1, c], c_sem.at[c])
            v_copy(0, c).start(priority=P_BULK)
            if c < len(wo_pcs):
                wo_copy(0, wo_pcs[c]).start(priority=P_SMALL)
            else:
                w3_copy(NQT).start(priority=P_SMALL)
            m_vec = qk_step(0, c, qb2, m_vec)

        def b_head(h, m_prev, last):
            par = h % 2
            qb2 = None if last else load_qb(h + 1)
            m_vec = acc = l_vec = None
            for c in range(NCH):
                wait_all(vbuf.at[par, c], c_sem.at[c])
                if not last:
                    v_copy(h + 1, c).start(priority=P_BULK)
                    if c < len(wo_pcs):
                        wo_copy(h + 1, wo_pcs[c]).start(priority=P_SMALL)
                    else:
                        w3_copy(NQT + 1 + h).start(priority=P_SMALL)
                else:
                    if c < len(tail_pcs):
                        r0, nr, k = tail_pcs[c]
                        w4_copy((r0, nr, 0, D), k).start(priority=P_BULK)
                    if c < len(e2_pcs):
                        w4_copy(e2_pcs[c], 0).start(priority=P_SMALL)
                if c == 0:
                    m = jnp.max(m_prev, axis=1, keepdims=True)
                    inv_l = load_inv_l()
                    y = y_ref[...]
                p = jnp.exp(s_ref[par, :, c * CL:(c + 1) * CL] - m)
                pr = vbuf[par, c].astype(F32) * p
                for g in range(CL // 128):
                    pg = pr[:, g * 128:(g + 1) * 128]
                    acc = pg if acc is None else acc + pg
                    lg = p[:, g * 128:(g + 1) * 128]
                    l_vec = lg if l_vec is None else l_vec + lg
                if not last:
                    m_vec = qk_step(h + 1, c, qb2, m_vec)
                if c < NOP:
                    y = oproj_piece(h, c, inv_l, y)
                if c == NOP - 1:
                    y_ref[...] = y
                if c == NCH - 2:
                    wait_all(wo_buf.at[h + 1], wo_sem.at[par])
                    if last:
                        wait_all(w3_buf, w3_sem.at[0])
            acc_ref[0:DH, :] = acc
            acc_ref[DH:DH + 8, :] = jnp.broadcast_to(l_vec, (8, 128))
            return m_vec

        m_vec = lax.fori_loop(0, H - 1, lambda h, m: b_head(h, m, False), m_vec)
        b_head(H - 1, m_vec, True)

        inv_l = load_inv_l()
        y = y_ref[...]
        for i in range(NOP):
            y = oproj_piece(H, i, inv_l, y)
        hh = x_buf[...].astype(F32) + jnp.sum(y, axis=0, keepdims=True)
        x1 = _ln(hh)
        yn = jnp.broadcast_to(_ln(x1), (8, D)).astype(BF16)
        g = jnp.dot(yn, w3_buf[...], preferred_element_type=F32)
        g = jax.nn.gelu(g, approximate=True).astype(BF16)
        res = hh + x1
        gcol = jnp.concatenate(
            [_col_bcast(g[0:1, v:v + 128].astype(F32)) for v in range(V0, FF, 128)],
            axis=0)
        gcol = jnp.concatenate([gcol] * (D // 128), axis=1)
        for k in range(NM):
            g0, n = groups[k]
            wait_all(w4_buf.at[pl.ds(g0, n), :], w4_sem.at[k])
            part = jnp.dot(g[:, g0:g0 + n], w4_buf[g0:g0 + n, :],
                           preferred_element_type=F32)
            res = res + part[0:1, :]
        z = None
        for k in range(NM, len(groups)):
            g0, n = groups[k]
            wait_all(w4_buf.at[pl.ds(g0, n), :], w4_sem.at[k])
            pr = w4_buf[g0:g0 + n, :].astype(F32) * gcol[g0 - V0:g0 - V0 + n, :]
            for i in range(n // 8):
                t = pr[i * 8:(i + 1) * 8, :]
                z = t if z is None else z + t
        res = res + jnp.sum(z, axis=0, keepdims=True)
        out_ref[...] = res.astype(out_ref.dtype)

    scratch = [
        pltpu.VMEM((H, NCH, DH, CL), BF16),
        pltpu.VMEM((2, NCH, DH, CL), BF16),
        pltpu.VMEM((D, HD), BF16),
        pltpu.VMEM((H + 1, DH, D), BF16),
        pltpu.VMEM((D, FF), BF16),
        pltpu.VMEM((FF, D), BF16),
        pltpu.VMEM((1, D), BF16),
        pltpu.VMEM((8, D), BF16),
        pltpu.VMEM((HD, 128), F32),
        pltpu.VMEM((2, 1, W), F32),
        pltpu.VMEM((DH + 8, 128), F32),
        pltpu.VMEM((8, D), F32),
        pltpu.SemaphoreType.DMA((NCH,)),
        pltpu.SemaphoreType.DMA((1,)),
        pltpu.SemaphoreType.DMA((2,)),
        pltpu.SemaphoreType.DMA((1,)),
        pltpu.SemaphoreType.DMA((len(groups),)),
        pltpu.SemaphoreType.DMA((1,)),
    ]
    return kernel, scratch


@jax.jit
def pallas_sequential_preLN__sliding_block_cached__mixer_s_mlp__decode_kernel(
    A_x: jax.Array,
    A_k_cache: jax.Array,
    A_v_cache: jax.Array,
    A_wq: jax.Array,
    A_wo: jax.Array,
    B_x: jax.Array,
    B_w1: jax.Array,
    B_w2: jax.Array,
    B_w3: jax.Array,
    B_w4: jax.Array,
):
    B, S, D = A_x.shape
    _, H, SK, DH = A_k_cache.shape
    FF = B_w3.shape[1]
    assert B == 1 and S == 1
    W = min(4096, max(256, SK // 4))

    kt = jnp.swapaxes(A_k_cache, 2, 3).reshape(H, DH, SK)
    vt = jnp.swapaxes(A_v_cache, 2, 3).reshape(H, DH, SK)
    x2 = A_x.reshape(1, D)

    kernel, scratch = _make_kernel(H, DH, SK, W, D, FF)
    out = pl.pallas_call(
        kernel,
        in_specs=[pl.BlockSpec(memory_space=pl.ANY)] * 7,
        out_specs=pl.BlockSpec(memory_space=pltpu.VMEM),
        out_shape=jax.ShapeDtypeStruct((1, D), A_x.dtype),
        scratch_shapes=scratch,
        compiler_params=pltpu.CompilerParams(
            vmem_limit_bytes=100 * 1024 * 1024,
            disable_bounds_checks=True,
            disable_semaphore_checks=True,
        ),
    )(x2, kt, vt, A_wq, A_wo, B_w3, B_w4)
    return out.reshape(B, S, D)
```

```python
import jax
import jax.numpy as jnp
from jax import lax
import jax.experimental.pallas as pl
import jax.experimental.pallas.tpu as pltpu

F32 = jnp.float32
BF16 = jnp.bfloat16

EPS = 1e-5
CL = 256
NSUB = CL // 128
P_BULK = 1
P_SMALL = 0
OR = 16
W4_EARLY = (192, 192)
W4_TAIL_ROWS = 128
W4_MXU_GROUPS = (1152, 256)
W4_VPU_GROUPS = (64, 64)


def _ln(v):
    m = jnp.mean(v, axis=-1, keepdims=True)
    c = v - m
    var = jnp.mean(c * c, axis=-1, keepdims=True)
    return c / jnp.sqrt(var + EPS)


def _pieces640(r_lo, r_hi):
    out = []
    for r in range(r_lo, r_hi, 64):
        out += [(r + i * 16, 16, 0, 512) for i in range(4)] + [(r, 64, 512, 128)]
    return out


def _col_bcast(row):
    eye = (lax.broadcasted_iota(jnp.int32, (128, 128), 0)
           == lax.broadcasted_iota(jnp.int32, (128, 128), 1))
    col = jnp.sum(jnp.where(eye, jnp.broadcast_to(row, (128, 128)), 0.0),
                  axis=1, keepdims=True)
    return jnp.broadcast_to(col, (128, 128))


def _make_kernel(H, DH, SK, W, D, FF):
    NCH = W // CL
    W0 = SK - W
    HD = H * DH
    NOP = DH // OR
    NQT = HD // 128
    scale = float(DH) ** -0.5
    assert (H, DH, NCH, D, FF) == (32, 192, 16, 640, 1536)

    NT = D // 128
    WOR = DH * NT
    NWO = WOR // 64
    e1_pcs = _pieces640(0, W4_EARLY[0])
    e2_pcs = _pieces640(W4_EARLY[0], sum(W4_EARLY))
    groups, r = [], 0
    for n in W4_MXU_GROUPS + W4_VPU_GROUPS:
        groups.append((r, n))
        r += n
    assert r == FF
    NM = len(W4_MXU_GROUPS)
    V0 = groups[NM][0]
    tail_pcs = []
    for k, (g0, n) in enumerate(groups):
        r = max(g0, sum(W4_EARLY))
        while r < g0 + n:
            nr = min(W4_TAIL_ROWS, g0 + n - r)
            tail_pcs.append((r, nr, k))
            r += nr
    assert len(tail_pcs) <= NCH

    def kernel(x_hbm, kt_hbm, vt_hbm, wq_hbm, wo_hbm, w3_hbm, w4_hbm, out_ref,
               kbuf, vbuf, wq_buf, wo_buf, w3_buf, w4_buf, x_buf, xn_ref, qb_ref,
               s_ref, acc_ref, y_ref,
               c_sem, wq_sem, wo_sem, w3_sem, w4_sem, x_sem):

        def al(v, m):
            return v if isinstance(v, int) else pl.multiple_of(v, m)

        def k_start(h, c):
            for j in range(NSUB):
                col = al(W0 + c * CL + j * 128, 128)
                pltpu.make_async_copy(
                    kt_hbm.at[h, :, pl.ds(col, 128)], kbuf.at[h, c, j],
                    c_sem.at[c]).start(priority=P_BULK)

        def v_start(h, c):
            for j in range(NSUB):
                col = W0 + c * CL + j * 128
                pltpu.make_async_copy(
                    vt_hbm.at[h, :, pl.ds(col, 128)], vbuf.at[h % 2, c, j],
                    c_sem.at[c]).start(priority=P_BULK)

        def wait_all(buf, sem):
            pltpu.make_async_copy(buf, buf, sem).wait()

        def wq_copy(rg, lb, lanes):
            row = al(rg * 8, 8)
            return pltpu.make_async_copy(
                wq_hbm.at[pl.ds(row, 8), pl.ds(lb * lanes, lanes)],
                wq_buf.at[pl.ds(row, 8), pl.ds(lb * lanes, lanes)], wq_sem.at[0])

        def wo_copy(h, i):
            row = al(h * WOR + i * 64, 64)
            return pltpu.make_async_copy(
                wo_hbm.at[pl.ds(row, 64), :],
                wo_buf.at[h + 1, pl.ds(i * 64, 64), :], wo_sem.at[h % 2])

        def w3_copy(i):
            row = al(i * 8, 8)
            return pltpu.make_async_copy(
                w3_hbm.at[pl.ds(row, 8), :], w3_buf.at[pl.ds(row, 8), :],
                w3_sem.at[0])

        def w4_copy(pc, k):
            r0, nr, c0, nc = pc
            return pltpu.make_async_copy(
                w4_hbm.at[pl.ds(r0, nr), pl.ds(c0, nc)],
                w4_buf.at[pl.ds(r0, nr), pl.ds(c0, nc)], w4_sem.at[k])

        def k_step(h, c):
            wait_all(kbuf.at[h, c], c_sem.at[c])
            k_start(h + 1, c)

        def q_row(j):
            col = al(j * 128, 128)
            q = jnp.dot(xn_ref[...], wq_buf[:, pl.ds(col, 128)],
                        preferred_element_type=F32)
            return q.astype(BF16).astype(F32) * scale

        def oproj_piece(slot, i, inv_l, y):
            r0 = i * OR
            o = jnp.sum(acc_ref[r0:r0 + OR, :], axis=1, keepdims=True) * inv_l
            o = jnp.broadcast_to(o, (OR, 128))
            w = wo_buf[slot, r0 * NT:(r0 + OR) * NT, :].astype(F32)
            for g in range(OR // 8):
                og = jnp.concatenate([o[g * 8:(g + 1) * 8, :]] * NT, axis=0)
                y = y + w[g * 8 * NT:(g + 1) * 8 * NT, :] * og
            return y

        def load_inv_l():
            l = jnp.sum(acc_ref[DH:DH + 1, :], axis=1, keepdims=True)
            return 1.0 / l

        def load_qb(h):
            return qb_ref[pl.ds(al(h * DH, 64), DH), :]

        def qk_step(h, c, qb, m_vec):
            for j in range(NSUB):
                s = jnp.sum(kbuf[h, c, j].astype(F32) * qb, axis=0, keepdims=True)
                lo = c * CL + j * 128
                s_ref[h % 2, :, lo:lo + 128] = s
                m_vec = s if m_vec is None else jnp.maximum(m_vec, s)
            return m_vec

        x_cp = pltpu.make_async_copy(x_hbm, x_buf, x_sem.at[0])
        x_cp.start(priority=P_SMALL)
        for c in range(NCH):
            k_start(0, c)

        acc_ref[0:DH, :] = jnp.zeros((DH, 128), F32)
        acc_ref[DH:DH + 8, :] = jnp.ones((8, 128), F32)
        wo_buf[0] = jnp.zeros((WOR, 128), BF16)
        y_ref[...] = jnp.zeros((8 * NT, 128), F32)

        def a_body(it, carry):
            for u in range(3 * NCH):
                k_step(it * 3 + u // NCH, u % NCH)
                wq_copy(it * 8 + u // 6, u % 6, 1024).start(priority=P_SMALL)
            return carry

        lax.fori_loop(0, 8, a_body, 0)
        for u in range(3 * NCH):
            k_step(24 + u // NCH, u % NCH)
            wq_copy(64 + u // 3, u % 3, 2048).start(priority=P_SMALL)

        e1 = list(e1_pcs)

        def e1_slot():
            if e1:
                w4_copy(e1.pop(0), 0).start(priority=P_SMALL)

        HQ = 27
        q0 = None
        for u in range(5):
            k_step(HQ, u)
            e1_slot()
            if u == 0:
                x_cp.wait()
                xn = _ln(x_buf[...].astype(F32))
                xn_ref[...] = jnp.broadcast_to(xn, (8, D)).astype(BF16)
            if u == 4:
                wait_all(wq_buf, wq_sem.at[0])
                q0 = q_row(0)

        def q_body(i, q):
            u = i + 5
            k_step(HQ + u // NCH, u % NCH)
            w3_copy(i).start(priority=P_SMALL)
            qb_ref[pl.ds(al(i * 128, 128), 128), :] = _col_bcast(q[0:1, :])
            return q_row(jnp.minimum(i + 1, NQT - 1))

        lax.fori_loop(0, NQT, q_body, q0)
        for u in range(5 + NQT, 4 * NCH):
            k_step(HQ + u // NCH, u % NCH)
            e1_slot()

        m_vec = None
        qb = load_qb(0)
        for c in range(NCH):
            wait_all(kbuf.at[H - 1, c], c_sem.at[c])
            v_start(0, c)
            if c < NWO:
                wo_copy(0, c).start(priority=P_SMALL)
            else:
                w3_copy(NQT).start(priority=P_SMALL)
            m_vec = qk_step(0, c, qb, m_vec)

        def b_head(h, m_prev, last):
            par = h % 2
            qb = None if last else load_qb(h + 1)
            m_vec = acc = l_vec = None
            for c in range(NCH):
                wait_all(vbuf.at[par, c], c_sem.at[c])
                if not last:
                    v_start(h + 1, c)
                    if c < NWO:
                        wo_copy(h + 1, c).start(priority=P_SMALL)
                    else:
                        w3_copy(NQT + 1 + h).start(priority=P_SMALL)
                else:
                    if c < len(tail_pcs):
                        r0, nr, k = tail_pcs[c]
                        w4_copy((r0, nr, 0, D), k).start(priority=P_BULK)
                    if c < len(e2_pcs):
                        w4_copy(e2_pcs[c], 0).start(priority=P_SMALL)
                if c == 0:
                    m = jnp.max(m_prev, axis=1, keepdims=True)
                    inv_l = load_inv_l()
                    y = y_ref[...]
                for j in range(NSUB):
                    lo = c * CL + j * 128
                    p = jnp.exp(s_ref[par, :, lo:lo + 128] - m)
                    pv = vbuf[par, c, j].astype(F32) * p
                    acc = pv if acc is None else acc + pv
                    l_vec = p if l_vec is None else l_vec + p
                if not last:
                    m_vec = qk_step(h + 1, c, qb, m_vec)
                if c < NOP:
                    y = oproj_piece(h, c, inv_l, y)
                if c == NOP - 1:
                    y_ref[...] = y
                if c == NCH - 2:
                    wait_all(wo_buf.at[h + 1], wo_sem.at[par])
                    if last:
                        wait_all(w3_buf, w3_sem.at[0])
            acc_ref[0:DH, :] = acc
            acc_ref[DH:DH + 8, :] = jnp.broadcast_to(l_vec, (8, 128))
            return m_vec

        m_vec = lax.fori_loop(0, H - 1, lambda h, m: b_head(h, m, False), m_vec)
        b_head(H - 1, m_vec, True)

        inv_l = load_inv_l()
        y = y_ref[...]
        for i in range(NOP):
            y = oproj_piece(H, i, inv_l, y)
        attn = jnp.concatenate(
            [jnp.sum(y[t * 8:(t + 1) * 8, :], axis=0, keepdims=True) for t in range(NT)],
            axis=1)
        hh = x_buf[...].astype(F32) + attn
        x1 = _ln(hh)
        yn = jnp.broadcast_to(_ln(x1), (8, D)).astype(BF16)
        g = jnp.dot(yn, w3_buf[...], preferred_element_type=F32)
        g = jax.nn.gelu(g, approximate=True).astype(BF16)
        res = hh + x1
        gcol = jnp.concatenate(
            [_col_bcast(g[0:1, v:v + 128].astype(F32)) for v in range(V0, FF, 128)],
            axis=0)
        gcol = jnp.concatenate([gcol] * (D // 128), axis=1)
        for k in range(NM):
            g0, n = groups[k]
            wait_all(w4_buf.at[pl.ds(g0, n), :], w4_sem.at[k])
            part = jnp.dot(g[:, g0:g0 + n], w4_buf[g0:g0 + n, :],
                           preferred_element_type=F32)
            res = res + part[0:1, :]
        z = None
        for k in range(NM, len(groups)):
            g0, n = groups[k]
            wait_all(w4_buf.at[pl.ds(g0, n), :], w4_sem.at[k])
            pr = w4_buf[g0:g0 + n, :].astype(F32) * gcol[g0 - V0:g0 - V0 + n, :]
            for i in range(n // 8):
                t = pr[i * 8:(i + 1) * 8, :]
                z = t if z is None else z + t
        res = res + jnp.sum(z, axis=0, keepdims=True)
        out_ref[...] = res.astype(out_ref.dtype)

    scratch = [
        pltpu.VMEM((H, NCH, NSUB, DH, 128), BF16),
        pltpu.VMEM((2, NCH, NSUB, DH, 128), BF16),
        pltpu.VMEM((D, HD), BF16),
        pltpu.VMEM((H + 1, WOR, 128), BF16),
        pltpu.VMEM((D, FF), BF16),
        pltpu.VMEM((FF, D), BF16),
        pltpu.VMEM((1, D), BF16),
        pltpu.VMEM((8, D), BF16),
        pltpu.VMEM((HD, 128), F32),
        pltpu.VMEM((2, 1, W), F32),
        pltpu.VMEM((DH + 8, 128), F32),
        pltpu.VMEM((8 * NT, 128), F32),
        pltpu.SemaphoreType.DMA((NCH,)),
        pltpu.SemaphoreType.DMA((1,)),
        pltpu.SemaphoreType.DMA((2,)),
        pltpu.SemaphoreType.DMA((1,)),
        pltpu.SemaphoreType.DMA((len(groups),)),
        pltpu.SemaphoreType.DMA((1,)),
    ]
    return kernel, scratch


@jax.jit
def pallas_sequential_preLN__sliding_block_cached__mixer_s_mlp__decode_kernel(
    A_x: jax.Array,
    A_k_cache: jax.Array,
    A_v_cache: jax.Array,
    A_wq: jax.Array,
    A_wo: jax.Array,
    B_x: jax.Array,
    B_w1: jax.Array,
    B_w2: jax.Array,
    B_w3: jax.Array,
    B_w4: jax.Array,
):
    B, S, D = A_x.shape
    _, H, SK, DH = A_k_cache.shape
    FF = B_w3.shape[1]
    assert B == 1 and S == 1
    W = min(4096, max(256, SK // 4))

    kt = jnp.swapaxes(A_k_cache, 2, 3).reshape(H, DH, SK)
    vt = jnp.swapaxes(A_v_cache, 2, 3).reshape(H, DH, SK)
    x2 = A_x.reshape(1, D)
    wo_t = A_wo.reshape(H * DH // 8, 8, D // 128, 128).transpose(0, 2, 1, 3)
    wo_t = wo_t.reshape(H * DH * (D // 128), 128)

    kernel, scratch = _make_kernel(H, DH, SK, W, D, FF)
    out = pl.pallas_call(
        kernel,
        in_specs=[pl.BlockSpec(memory_space=pl.ANY)] * 7,
        out_specs=pl.BlockSpec(memory_space=pltpu.VMEM),
        out_shape=jax.ShapeDtypeStruct((1, D), A_x.dtype),
        scratch_shapes=scratch,
        compiler_params=pltpu.CompilerParams(
            vmem_limit_bytes=100 * 1024 * 1024,
            disable_bounds_checks=True,
            disable_semaphore_checks=True,
        ),
    )(x2, kt, vt, A_wq, wo_t, B_w3, B_w4)
    return out.reshape(B, S, D)
```

```python
import jax
import jax.numpy as jnp
from jax import lax
import jax.experimental.pallas as pl
import jax.experimental.pallas.tpu as pltpu

F32 = jnp.float32
BF16 = jnp.bfloat16

EPS = 1e-5
CL = 256
NSUB = CL // 128
SUBS = tuple(range(NSUB))
P_BULK = 1
P_SMALL = 0
OR = 16
W4_EARLY = (192, 192)
W4_TAIL_ROWS = 128
W4_MXU_GROUPS = (1152, 256)
W4_VPU_GROUPS = (64, 64)


def _ln(v):
    m = jnp.mean(v, axis=-1, keepdims=True)
    c = v - m
    var = jnp.mean(c * c, axis=-1, keepdims=True)
    return c / jnp.sqrt(var + EPS)


def _pieces640(r_lo, r_hi):
    out = []
    for r in range(r_lo, r_hi, 64):
        out += [(r + i * 16, 16, 0, 512) for i in range(4)] + [(r, 64, 512, 128)]
    return out


def _col_bcast(row):
    eye = (lax.broadcasted_iota(jnp.int32, (128, 128), 0)
           == lax.broadcasted_iota(jnp.int32, (128, 128), 1))
    col = jnp.sum(jnp.where(eye, jnp.broadcast_to(row, (128, 128)), 0.0),
                  axis=1, keepdims=True)
    return jnp.broadcast_to(col, (128, 128))


def _make_kernel(H, DH, SK, W, D, FF):
    NCH = W // CL
    W0 = SK - W
    HD = H * DH
    NOP = DH // OR
    NQT = HD // 128
    scale = float(DH) ** -0.5
    assert (H, DH, NCH, D, FF) == (32, 192, 16, 640, 1536)

    NT = D // 128
    WOR = DH * NT
    NWO = WOR // 64
    e1_pcs = _pieces640(0, W4_EARLY[0])
    e2_pcs = _pieces640(W4_EARLY[0], sum(W4_EARLY))
    groups, r = [], 0
    for n in W4_MXU_GROUPS + W4_VPU_GROUPS:
        groups.append((r, n))
        r += n
    assert r == FF
    NM = len(W4_MXU_GROUPS)
    V0 = groups[NM][0]
    tail_pcs = []
    for k, (g0, n) in enumerate(groups):
        r = max(g0, sum(W4_EARLY))
        while r < g0 + n:
            nr = min(W4_TAIL_ROWS, g0 + n - r)
            tail_pcs.append((r, nr, k))
            r += nr
    assert len(tail_pcs) <= NCH

    def kernel(x_hbm, kt_hbm, vt_hbm, wq_hbm, wo_hbm, w3_hbm, w4_hbm, out_ref,
               kbuf, vbuf, wq_buf, wo_buf, w3_buf, w4_buf, x_buf, xn_ref, qb_ref,
               s_ref, acc_ref, y_ref,
               c_sem, wq_sem, wo_sem, w3_sem, w4_sem, x_sem):

        def al(v, m):
            return v if isinstance(v, int) else pl.multiple_of(v, m)

        def k_start(h, c, js=SUBS):
            for j in js:
                col = al(W0 + c * CL + j * 128, 128)
                pltpu.make_async_copy(
                    kt_hbm.at[h, :, pl.ds(col, 128)], kbuf.at[h, c, j],
                    c_sem.at[NSUB * c + j]).start(priority=P_BULK)

        def v_start(h, c):
            for j in SUBS:
                col = W0 + c * CL + j * 128
                pltpu.make_async_copy(
                    vt_hbm.at[h, :, pl.ds(col, 128)], vbuf.at[h % 2, c, j],
                    c_sem.at[NSUB * c + j]).start(priority=P_BULK)

        def wait_all(buf, sem):
            pltpu.make_async_copy(buf, buf, sem).wait()

        def c_wait(buf, i, c, js=SUBS):
            for j in js:
                wait_all(buf.at[i, c, j], c_sem.at[NSUB * c + j])

        def wq_copy(rg, lb, lanes):
            row = al(rg * 8, 8)
            return pltpu.make_async_copy(
                wq_hbm.at[pl.ds(row, 8), pl.ds(lb * lanes, lanes)],
                wq_buf.at[pl.ds(row, 8), pl.ds(lb * lanes, lanes)], wq_sem.at[0])

        def wo_copy(h, i):
            row = al(h * WOR + i * 64, 64)
            return pltpu.make_async_copy(
                wo_hbm.at[pl.ds(row, 64), :],
                wo_buf.at[h + 1, pl.ds(i * 64, 64), :], wo_sem.at[h % 2])

        def w3_copy(i):
            row = al(i * 8, 8)
            return pltpu.make_async_copy(
                w3_hbm.at[pl.ds(row, 8), :], w3_buf.at[pl.ds(row, 8), :],
                w3_sem.at[0])

        def w4_copy(pc, k):
            r0, nr, c0, nc = pc
            return pltpu.make_async_copy(
                w4_hbm.at[pl.ds(r0, nr), pl.ds(c0, nc)],
                w4_buf.at[pl.ds(r0, nr), pl.ds(c0, nc)], w4_sem.at[k])

        def k_step(h, c, js=SUBS):
            c_wait(kbuf, h, c, js)
            k_start(h + 1, c, js)

        def q_row(j):
            col = al(j * 128, 128)
            q = jnp.dot(xn_ref[...], wq_buf[:, pl.ds(col, 128)],
                        preferred_element_type=F32)
            return q.astype(BF16).astype(F32) * scale

        def oproj_piece(slot, i, inv_l, y):
            r0 = i * OR
            o = jnp.sum(acc_ref[r0:r0 + OR, :], axis=1, keepdims=True) * inv_l
            o = jnp.broadcast_to(o, (OR, 128))
            w = wo_buf[slot, r0 * NT:(r0 + OR) * NT, :].astype(F32)
            for g in range(OR // 8):
                og = jnp.concatenate([o[g * 8:(g + 1) * 8, :]] * NT, axis=0)
                y = y + w[g * 8 * NT:(g + 1) * 8 * NT, :] * og
            return y

        def load_inv_l():
            l = jnp.sum(acc_ref[DH:DH + 1, :], axis=1, keepdims=True)
            return 1.0 / l

        def load_qb(h):
            return qb_ref[pl.ds(al(h * DH, 64), DH), :]

        def qk_step(h, c, qb, m_vec):
            for j in SUBS:
                s = jnp.sum(kbuf[h, c, j].astype(F32) * qb, axis=0, keepdims=True)
                lo = c * CL + j * 128
                s_ref[h % 2, :, lo:lo + 128] = s
                m_vec = s if m_vec is None else jnp.maximum(m_vec, s)
            return m_vec

        x_cp = pltpu.make_async_copy(x_hbm, x_buf, x_sem.at[0])
        x_cp.start(priority=P_SMALL)
        for c in range(NCH):
            k_start(0, c)

        acc_ref[0:DH, :] = jnp.zeros((DH, 128), F32)
        acc_ref[DH:DH + 8, :] = jnp.ones((8, 128), F32)
        wo_buf[0] = jnp.zeros((WOR, 128), BF16)
        y_ref[...] = jnp.zeros((8 * NT, 128), F32)

        def a_steps(h0, rg0, lanes):
            per_rg = HD // lanes
            for u in range(3 * NCH * NSUB):
                v = u // NSUB
                k_step(h0 + v // NCH, v % NCH, (u % NSUB,))
                wq_copy(rg0 + u // per_rg, u % per_rg, lanes).start(priority=P_SMALL)

        def a_body(it, carry):
            a_steps(it * 3, it * 8, 512)
            return carry

        lax.fori_loop(0, 8, a_body, 0)
        a_steps(24, 64, 1024)

        e1 = list(e1_pcs)

        def e1_slot():
            if e1:
                w4_copy(e1.pop(0), 0).start(priority=P_SMALL)

        HQ = 27
        q0 = None
        for u in range(5):
            k_step(HQ, u)
            e1_slot()
            if u == 0:
                x_cp.wait()
                xn = _ln(x_buf[...].astype(F32))
                xn_ref[...] = jnp.broadcast_to(xn, (8, D)).astype(BF16)
            if u == 4:
                wait_all(wq_buf, wq_sem.at[0])
                q0 = q_row(0)

        def q_body(i, q):
            u = i + 5
            k_step(HQ + u // NCH, u % NCH)
            w3_copy(i).start(priority=P_SMALL)
            qb_ref[pl.ds(al(i * 128, 128), 128), :] = _col_bcast(q[0:1, :])
            return q_row(jnp.minimum(i + 1, NQT - 1))

        lax.fori_loop(0, NQT, q_body, q0)
        for u in range(5 + NQT, 4 * NCH):
            k_step(HQ + u // NCH, u % NCH)
            e1_slot()

        m_vec = None
        qb = load_qb(0)
        for c in range(NCH):
            c_wait(kbuf, H - 1, c)
            v_start(0, c)
            if c < NWO:
                wo_copy(0, c).start(priority=P_SMALL)
            else:
                w3_copy(NQT).start(priority=P_SMALL)
            m_vec = qk_step(0, c, qb, m_vec)

        def b_head(h, m_prev, last):
            par = h % 2
            qb = None if last else load_qb(h + 1)
            m_vec = acc = l_vec = None
            for c in range(NCH):
                c_wait(vbuf, par, c)
                if not last:
                    v_start(h + 1, c)
                    if c < NWO:
                        wo_copy(h + 1, c).start(priority=P_SMALL)
                    else:
                        w3_copy(NQT + 1 + h).start(priority=P_SMALL)
                else:
                    if c < len(tail_pcs):
                        r0, nr, k = tail_pcs[c]
                        w4_copy((r0, nr, 0, D), k).start(priority=P_BULK)
                    if c < len(e2_pcs):
                        w4_copy(e2_pcs[c], 0).start(priority=P_SMALL)
                if c == 0:
                    m = jnp.max(m_prev, axis=1, keepdims=True)
                    inv_l = load_inv_l()
                    y = y_ref[...]
                for j in SUBS:
                    lo = c * CL + j * 128
                    p = jnp.exp(s_ref[par, :, lo:lo + 128] - m)
                    pv = vbuf[par, c, j].astype(F32) * p
                    acc = pv if acc is None else acc + pv
                    l_vec = p if l_vec is None else l_vec + p
                if not last:
                    m_vec = qk_step(h + 1, c, qb, m_vec)
                if c < NOP:
                    y = oproj_piece(h, c, inv_l, y)
                if c == NOP - 1:
                    y_ref[...] = y
                if c == NCH - 2:
                    wait_all(wo_buf.at[h + 1], wo_sem.at[par])
                    if last:
                        wait_all(w3_buf, w3_sem.at[0])
            acc_ref[0:DH, :] = acc
            acc_ref[DH:DH + 8, :] = jnp.broadcast_to(l_vec, (8, 128))
            return m_vec

        m_vec = lax.fori_loop(0, H - 1, lambda h, m: b_head(h, m, False), m_vec)
        b_head(H - 1, m_vec, True)

        inv_l = load_inv_l()
        y = y_ref[...]
        for i in range(NOP):
            y = oproj_piece(H, i, inv_l, y)
        attn = jnp.concatenate(
            [jnp.sum(y[t * 8:(t + 1) * 8, :], axis=0, keepdims=True) for t in range(NT)],
            axis=1)
        hh = x_buf[...].astype(F32) + attn
        x1 = _ln(hh)
        yn = jnp.broadcast_to(_ln(x1), (8, D)).astype(BF16)
        g = jnp.dot(yn, w3_buf[...], preferred_element_type=F32)
        g = jax.nn.gelu(g, approximate=True).astype(BF16)
        res = hh + x1
        gcol = jnp.concatenate(
            [_col_bcast(g[0:1, v:v + 128].astype(F32)) for v in range(V0, FF, 128)],
            axis=0)
        gcol = jnp.concatenate([gcol] * (D // 128), axis=1)
        for k in range(NM):
            g0, n = groups[k]
            wait_all(w4_buf.at[pl.ds(g0, n), :], w4_sem.at[k])
            part = jnp.dot(g[:, g0:g0 + n], w4_buf[g0:g0 + n, :],
                           preferred_element_type=F32)
            res = res + part[0:1, :]
        z = None
        for k in range(NM, len(groups)):
            g0, n = groups[k]
            wait_all(w4_buf.at[pl.ds(g0, n), :], w4_sem.at[k])
            pr = w4_buf[g0:g0 + n, :].astype(F32) * gcol[g0 - V0:g0 - V0 + n, :]
            for i in range(n // 8):
                t = pr[i * 8:(i + 1) * 8, :]
                z = t if z is None else z + t
        res = res + jnp.sum(z, axis=0, keepdims=True)
        out_ref[...] = res.astype(out_ref.dtype)

    scratch = [
        pltpu.VMEM((H, NCH, NSUB, DH, 128), BF16),
        pltpu.VMEM((2, NCH, NSUB, DH, 128), BF16),
        pltpu.VMEM((D, HD), BF16),
        pltpu.VMEM((H + 1, WOR, 128), BF16),
        pltpu.VMEM((D, FF), BF16),
        pltpu.VMEM((FF, D), BF16),
        pltpu.VMEM((1, D), BF16),
        pltpu.VMEM((8, D), BF16),
        pltpu.VMEM((HD, 128), F32),
        pltpu.VMEM((2, 1, W), F32),
        pltpu.VMEM((DH + 8, 128), F32),
        pltpu.VMEM((8 * NT, 128), F32),
        pltpu.SemaphoreType.DMA((NCH * NSUB,)),
        pltpu.SemaphoreType.DMA((1,)),
        pltpu.SemaphoreType.DMA((2,)),
        pltpu.SemaphoreType.DMA((1,)),
        pltpu.SemaphoreType.DMA((len(groups),)),
        pltpu.SemaphoreType.DMA((1,)),
    ]
    return kernel, scratch


@jax.jit
def pallas_sequential_preLN__sliding_block_cached__mixer_s_mlp__decode_kernel(
    A_x: jax.Array,
    A_k_cache: jax.Array,
    A_v_cache: jax.Array,
    A_wq: jax.Array,
    A_wo: jax.Array,
    B_x: jax.Array,
    B_w1: jax.Array,
    B_w2: jax.Array,
    B_w3: jax.Array,
    B_w4: jax.Array,
):
    B, S, D = A_x.shape
    _, H, SK, DH = A_k_cache.shape
    FF = B_w3.shape[1]
    assert B == 1 and S == 1
    W = min(4096, max(256, SK // 4))

    kt = jnp.swapaxes(A_k_cache, 2, 3).reshape(H, DH, SK)
    vt = jnp.swapaxes(A_v_cache, 2, 3).reshape(H, DH, SK)
    x2 = A_x.reshape(1, D)
    wo_t = A_wo.reshape(H * DH // 8, 8, D // 128, 128).transpose(0, 2, 1, 3)
    wo_t = wo_t.reshape(H * DH * (D // 128), 128)

    kernel, scratch = _make_kernel(H, DH, SK, W, D, FF)
    out = pl.pallas_call(
        kernel,
        in_specs=[pl.BlockSpec(memory_space=pl.ANY)] * 7,
        out_specs=pl.BlockSpec(memory_space=pltpu.VMEM),
        out_shape=jax.ShapeDtypeStruct((1, D), A_x.dtype),
        scratch_shapes=scratch,
        compiler_params=pltpu.CompilerParams(
            vmem_limit_bytes=100 * 1024 * 1024,
            disable_bounds_checks=True,
            disable_semaphore_checks=True,
        ),
    )(x2, kt, vt, A_wq, wo_t, B_w3, B_w4)
    return out.reshape(B, S, D)
```

```python
import jax
import jax.numpy as jnp
from jax import lax
import jax.experimental.pallas as pl
import jax.experimental.pallas.tpu as pltpu

F32 = jnp.float32
BF16 = jnp.bfloat16

EPS = 1e-5
CL = 256
NSUB = CL // 128
SUBS = tuple(range(NSUB))
P_BULK = 1
P_SMALL = 0
OR = 16
W4_EARLY = (192, 192)
W4_TAIL_ROWS = 128
W4_MXU_GROUPS = (1152, 256)
W4_VPU_GROUPS = (64, 64)


def _ln(v):
    m = jnp.mean(v, axis=-1, keepdims=True)
    c = v - m
    var = jnp.mean(c * c, axis=-1, keepdims=True)
    return c / jnp.sqrt(var + EPS)


def _pieces640(r_lo, r_hi):
    out = []
    for r in range(r_lo, r_hi, 64):
        out += [(r + i * 16, 16, 0, 512) for i in range(4)] + [(r, 64, 512, 128)]
    return out


def _col_bcast(row):
    eye = (lax.broadcasted_iota(jnp.int32, (128, 128), 0)
           == lax.broadcasted_iota(jnp.int32, (128, 128), 1))
    col = jnp.sum(jnp.where(eye, jnp.broadcast_to(row, (128, 128)), 0.0),
                  axis=1, keepdims=True)
    return jnp.broadcast_to(col, (128, 128))


def _make_kernel(H, DH, SK, W, D, FF):
    NCH = W // CL
    W0 = SK - W
    HD = H * DH
    NOP = DH // OR
    NQT = HD // 128
    scale = float(DH) ** -0.5
    assert (H, DH, NCH, D, FF) == (32, 192, 16, 640, 1536)

    NT = D // 128
    WOR = DH * NT
    NWO = WOR // 64
    e1_pcs = _pieces640(0, W4_EARLY[0])
    e2_pcs = _pieces640(W4_EARLY[0], sum(W4_EARLY))
    groups, r = [], 0
    for n in W4_MXU_GROUPS + W4_VPU_GROUPS:
        groups.append((r, n))
        r += n
    assert r == FF
    NM = len(W4_MXU_GROUPS)
    V0 = groups[NM][0]
    tail_pcs = []
    for k, (g0, n) in enumerate(groups):
        r = max(g0, sum(W4_EARLY))
        while r < g0 + n:
            nr = min(W4_TAIL_ROWS, g0 + n - r)
            tail_pcs.append((r, nr, k))
            r += nr
    assert len(tail_pcs) <= NCH

    def kernel(x_hbm, kt_hbm, vt_hbm, wq_hbm, wo_hbm, w3_hbm, w4_hbm, out_ref,
               kbuf, vbuf, wq_buf, wo_buf, w3_buf, w4_buf, x_buf, xn_ref, qb_ref,
               s_ref, acc_ref, y_ref,
               c_sem, wq_sem, wo_sem, w3_sem, w4_sem, x_sem):

        def al(v, m):
            return v if isinstance(v, int) else pl.multiple_of(v, m)

        def k_start(h, c, js=SUBS):
            for j in js:
                col = al(W0 + c * CL + j * 128, 128)
                pltpu.make_async_copy(
                    kt_hbm.at[h, :, pl.ds(col, 128)], kbuf.at[h, c, j],
                    c_sem.at[NSUB * c + j]).start(priority=P_BULK)

        def v_start(h, c):
            for j in SUBS:
                col = W0 + c * CL + j * 128
                pltpu.make_async_copy(
                    vt_hbm.at[h, :, pl.ds(col, 128)], vbuf.at[h % 2, c, j],
                    c_sem.at[NSUB * c + j]).start(priority=P_BULK)

        def wait_all(buf, sem):
            pltpu.make_async_copy(buf, buf, sem).wait()

        def c_wait(buf, i, c, js=SUBS):
            for j in js:
                wait_all(buf.at[i, c, j], c_sem.at[NSUB * c + j])

        def wq_copy(rg, lb, nt):
            return pltpu.make_async_copy(
                wq_hbm.at[rg, pl.ds(lb * nt, nt)],
                wq_buf.at[pl.ds(lb * nt, nt), pl.ds(al(rg * 8, 8), 8), :],
                wq_sem.at[0])

        def wo_copy(h, i):
            row = al(h * WOR + i * 64, 64)
            return pltpu.make_async_copy(
                wo_hbm.at[pl.ds(row, 64), :],
                wo_buf.at[h + 1, pl.ds(i * 64, 64), :], wo_sem.at[h % 2])

        def w3_copy(i):
            row = al(i * 8, 8)
            return pltpu.make_async_copy(
                w3_hbm.at[pl.ds(row, 8), :], w3_buf.at[pl.ds(row, 8), :],
                w3_sem.at[0])

        def w4_copy(pc, k):
            r0, nr, c0, nc = pc
            return pltpu.make_async_copy(
                w4_hbm.at[pl.ds(r0, nr), pl.ds(c0, nc)],
                w4_buf.at[pl.ds(r0, nr), pl.ds(c0, nc)], w4_sem.at[k])

        def k_step(h, c, js=SUBS):
            c_wait(kbuf, h, c, js)
            k_start(h + 1, c, js)

        def q_row(j):
            q = jnp.dot(xn_ref[...], wq_buf[j],
                        preferred_element_type=F32)
            return q.astype(BF16).astype(F32) * scale

        def oproj_piece(slot, i, inv_l, y):
            r0 = i * OR
            o = jnp.sum(acc_ref[r0:r0 + OR, :], axis=1, keepdims=True) * inv_l
            o = jnp.broadcast_to(o, (OR, 128))
            w = wo_buf[slot, r0 * NT:(r0 + OR) * NT, :].astype(F32)
            for g in range(OR // 8):
                og = jnp.concatenate([o[g * 8:(g + 1) * 8, :]] * NT, axis=0)
                y = y + w[g * 8 * NT:(g + 1) * 8 * NT, :] * og
            return y

        def load_inv_l():
            l = jnp.sum(acc_ref[DH:DH + 1, :], axis=1, keepdims=True)
            return 1.0 / l

        def load_qb(h):
            return qb_ref[pl.ds(al(h * DH, 64), DH), :]

        def qk_step(h, c, qb, m_vec):
            for j in SUBS:
                s = jnp.sum(kbuf[h, c, j].astype(F32) * qb, axis=0, keepdims=True)
                lo = c * CL + j * 128
                s_ref[h % 2, :, lo:lo + 128] = s
                m_vec = s if m_vec is None else jnp.maximum(m_vec, s)
            return m_vec

        x_cp = pltpu.make_async_copy(x_hbm, x_buf, x_sem.at[0])
        x_cp.start(priority=P_SMALL)
        for c in range(NCH):
            k_start(0, c)

        acc_ref[0:DH, :] = jnp.zeros((DH, 128), F32)
        acc_ref[DH:DH + 8, :] = jnp.ones((8, 128), F32)
        wo_buf[0] = jnp.zeros((WOR, 128), BF16)
        y_ref[...] = jnp.zeros((8 * NT, 128), F32)

        def a_steps(h0, rg0, nt):
            per_rg = NQT // nt
            for u in range(3 * NCH * NSUB):
                v = u // NSUB
                k_step(h0 + v // NCH, v % NCH, (u % NSUB,))
                wq_copy(rg0 + u // per_rg, u % per_rg, nt).start(priority=P_SMALL)

        def a_body(it, carry):
            a_steps(it * 3, it * 8, 4)
            return carry

        lax.fori_loop(0, 8, a_body, 0)
        a_steps(24, 64, 8)

        e1 = list(e1_pcs)

        def e1_slot():
            if e1:
                w4_copy(e1.pop(0), 0).start(priority=P_SMALL)

        HQ = 27
        q0 = None
        for u in range(5):
            k_step(HQ, u)
            e1_slot()
            if u == 0:
                x_cp.wait()
                xn = _ln(x_buf[...].astype(F32))
                xn_ref[...] = jnp.broadcast_to(xn, (8, D)).astype(BF16)
            if u == 4:
                wait_all(wq_buf, wq_sem.at[0])
                q0 = q_row(0)

        def q_body(i, q):
            u = i + 5
            k_step(HQ + u // NCH, u % NCH)
            w3_copy(i).start(priority=P_SMALL)
            qb_ref[pl.ds(al(i * 128, 128), 128), :] = _col_bcast(q[0:1, :])
            return q_row(jnp.minimum(i + 1, NQT - 1))

        lax.fori_loop(0, NQT, q_body, q0)
        for u in range(5 + NQT, 4 * NCH):
            k_step(HQ + u // NCH, u % NCH)
            e1_slot()

        m_vec = None
        qb = load_qb(0)
        for c in range(NCH):
            c_wait(kbuf, H - 1, c)
            v_start(0, c)
            if c < NWO:
                wo_copy(0, c).start(priority=P_SMALL)
            else:
                w3_copy(NQT).start(priority=P_SMALL)
            m_vec = qk_step(0, c, qb, m_vec)

        def b_head(h, m_prev, last):
            par = h % 2
            qb = None if last else load_qb(h + 1)
            m_vec = acc = l_vec = None
            for c in range(NCH):
                c_wait(vbuf, par, c)
                if not last:
                    v_start(h + 1, c)
                    if c < NWO:
                        wo_copy(h + 1, c).start(priority=P_SMALL)
                    else:
                        w3_copy(NQT + 1 + h).start(priority=P_SMALL)
                else:
                    if c < len(tail_pcs):
                        r0, nr, k = tail_pcs[c]
                        w4_copy((r0, nr, 0, D), k).start(priority=P_BULK)
                    if c < len(e2_pcs):
                        w4_copy(e2_pcs[c], 0).start(priority=P_SMALL)
                if c == 0:
                    m = jnp.max(m_prev, axis=1, keepdims=True)
                    inv_l = load_inv_l()
                    y = y_ref[...]
                for j in SUBS:
                    lo = c * CL + j * 128
                    p = jnp.exp(s_ref[par, :, lo:lo + 128] - m)
                    pv = vbuf[par, c, j].astype(F32) * p
                    acc = pv if acc is None else acc + pv
                    l_vec = p if l_vec is None else l_vec + p
                if not last:
                    m_vec = qk_step(h + 1, c, qb, m_vec)
                if c < NOP:
                    y = oproj_piece(h, c, inv_l, y)
                if c == NOP - 1:
                    y_ref[...] = y
                if c == NCH - 2:
                    wait_all(wo_buf.at[h + 1], wo_sem.at[par])
                    if last:
                        wait_all(w3_buf, w3_sem.at[0])
            acc_ref[0:DH, :] = acc
            acc_ref[DH:DH + 8, :] = jnp.broadcast_to(l_vec, (8, 128))
            return m_vec

        m_vec = lax.fori_loop(0, H - 1, lambda h, m: b_head(h, m, False), m_vec)
        b_head(H - 1, m_vec, True)

        inv_l = load_inv_l()
        y = y_ref[...]
        for i in range(NOP):
            y = oproj_piece(H, i, inv_l, y)
        attn = jnp.concatenate(
            [jnp.sum(y[t * 8:(t + 1) * 8, :], axis=0, keepdims=True) for t in range(NT)],
            axis=1)
        hh = x_buf[...].astype(F32) + attn
        x1 = _ln(hh)
        yn = jnp.broadcast_to(_ln(x1), (8, D)).astype(BF16)
        g = jnp.dot(yn, w3_buf[...], preferred_element_type=F32)
        g = jax.nn.gelu(g, approximate=True).astype(BF16)
        res = hh + x1
        gcol = jnp.concatenate(
            [_col_bcast(g[0:1, v:v + 128].astype(F32)) for v in range(V0, FF, 128)],
            axis=0)
        gcol = jnp.concatenate([gcol] * (D // 128), axis=1)
        for k in range(NM):
            g0, n = groups[k]
            wait_all(w4_buf.at[pl.ds(g0, n), :], w4_sem.at[k])
            part = jnp.dot(g[:, g0:g0 + n], w4_buf[g0:g0 + n, :],
                           preferred_element_type=F32)
            res = res + part[0:1, :]
        z = None
        for k in range(NM, len(groups)):
            g0, n = groups[k]
            wait_all(w4_buf.at[pl.ds(g0, n), :], w4_sem.at[k])
            pr = w4_buf[g0:g0 + n, :].astype(F32) * gcol[g0 - V0:g0 - V0 + n, :]
            for i in range(n // 8):
                t = pr[i * 8:(i + 1) * 8, :]
                z = t if z is None else z + t
        res = res + jnp.sum(z, axis=0, keepdims=True)
        out_ref[...] = res.astype(out_ref.dtype)

    scratch = [
        pltpu.VMEM((H, NCH, NSUB, DH, 128), BF16),
        pltpu.VMEM((2, NCH, NSUB, DH, 128), BF16),
        pltpu.VMEM((NQT, D, 128), BF16),
        pltpu.VMEM((H + 1, WOR, 128), BF16),
        pltpu.VMEM((D, FF), BF16),
        pltpu.VMEM((FF, D), BF16),
        pltpu.VMEM((1, D), BF16),
        pltpu.VMEM((8, D), BF16),
        pltpu.VMEM((HD, 128), F32),
        pltpu.VMEM((2, 1, W), F32),
        pltpu.VMEM((DH + 8, 128), F32),
        pltpu.VMEM((8 * NT, 128), F32),
        pltpu.SemaphoreType.DMA((NCH * NSUB,)),
        pltpu.SemaphoreType.DMA((1,)),
        pltpu.SemaphoreType.DMA((2,)),
        pltpu.SemaphoreType.DMA((1,)),
        pltpu.SemaphoreType.DMA((len(groups),)),
        pltpu.SemaphoreType.DMA((1,)),
    ]
    return kernel, scratch


@jax.jit
def pallas_sequential_preLN__sliding_block_cached__mixer_s_mlp__decode_kernel(
    A_x: jax.Array,
    A_k_cache: jax.Array,
    A_v_cache: jax.Array,
    A_wq: jax.Array,
    A_wo: jax.Array,
    B_x: jax.Array,
    B_w1: jax.Array,
    B_w2: jax.Array,
    B_w3: jax.Array,
    B_w4: jax.Array,
):
    B, S, D = A_x.shape
    _, H, SK, DH = A_k_cache.shape
    FF = B_w3.shape[1]
    assert B == 1 and S == 1
    W = min(4096, max(256, SK // 4))

    kt = jnp.swapaxes(A_k_cache, 2, 3).reshape(H, DH, SK)
    vt = jnp.swapaxes(A_v_cache, 2, 3).reshape(H, DH, SK)
    x2 = A_x.reshape(1, D)
    wq_t = A_wq.reshape(D // 8, 8, H * DH // 128, 128).transpose(0, 2, 1, 3)
    wo_t = A_wo.reshape(H * DH // 8, 8, D // 128, 128).transpose(0, 2, 1, 3)
    wo_t = wo_t.reshape(H * DH * (D // 128), 128)

    kernel, scratch = _make_kernel(H, DH, SK, W, D, FF)
    out = pl.pallas_call(
        kernel,
        in_specs=[pl.BlockSpec(memory_space=pl.ANY)] * 7,
        out_specs=pl.BlockSpec(memory_space=pltpu.VMEM),
        out_shape=jax.ShapeDtypeStruct((1, D), A_x.dtype),
        scratch_shapes=scratch,
        compiler_params=pltpu.CompilerParams(
            vmem_limit_bytes=100 * 1024 * 1024,
            disable_bounds_checks=True,
            disable_semaphore_checks=True,
        ),
    )(x2, kt, vt, wq_t, wo_t, B_w3, B_w4)
    return out.reshape(B, S, D)
```
